```python
import jax
import jax.numpy as jnp

def _softmax(x, axis=-1):
    return jax.nn.softmax(x, axis=axis)

def _gelu(x):
    return jax.nn.gelu(x, approximate=True)

def _silu(x):
    return jax.nn.silu(x)

def _sigmoid(x):
    return jax.nn.sigmoid(x)

def _layernorm(x, axis=-1, eps=1e-05):
    m = jnp.mean(x, axis=axis, keepdims=True)
    v = jnp.var(x, axis=axis, keepdims=True)
    return (x - m) / jnp.sqrt(v + eps)

def _scatter_add(tgt, idx, src, axis=0):
    return tgt.at[idx].add(src)

def _segment_sum(src, seg, n):
    return jax.ops.segment_sum(src, seg, n)

class _Rng:

    def __init__(self, key):
        self._k = key

    def _next(self):
        self._k, sub = jax.random.split(self._k)
        return sub

    def normal(self, shape):
        return jax.random.normal(self._next(), shape, dtype=jnp.bfloat16)

    def randint(self, lo, hi, shape):
        return jax.random.randint(self._next(), shape, lo, hi, dtype=jnp.int32)

    def uniform(self, shape, lo=0.0, hi=1.0):
        return jax.random.uniform(self._next(), shape, jnp.bfloat16, lo, hi)

    def permutation(self, n):
        return jax.random.permutation(self._next(), n)
kernel_name = 'adaLN_cond__sliding_block_cached__glu_gated_glu__decode'

def setup_inputs():
    _rng = _Rng(jax.random.key(int.from_bytes(__import__("os").urandom(4), "little")))
    _w = lambda a: (lambda t: t.astype(jnp.bfloat16) if jnp.issubdtype(t.dtype, jnp.floating) else t)(jnp.asarray(a))

    def _A_setup():
        B, Sq, D = (8, 1, 512)
        Hq, Hkv, Sk, Dh = (32, 32, 4096, 128)
        assert Hq % Hkv == 0, (Hq, Hkv)
        return {'x': _w((lambda *s: _rng.normal(s) * 0.05)(B, Sq, D)), 'k_cache': _w((lambda *s: _rng.normal(s) * 0.05)(B, Hkv, Sk, Dh)), 'v_cache': _w((lambda *s: _rng.normal(s) * 0.05)(B, Hkv, Sk, Dh)), 'wq': _w((lambda *s: _rng.normal(s) * 0.05)(D, Hq * Dh) * D ** (-0.5)), 'wo': _w((lambda *s: _rng.normal(s) * 0.05)(Hq * Dh, D) * (Hq * Dh) ** (-0.5))}
    _A_in = _A_setup()

    def _B_setup():
        B, S, D, F = (8, 1, 512, 1376)
        return {'x': _w((lambda *s: _rng.normal(s) * 0.05)(B, S, D)), 'w_gate': _w((lambda *s: _rng.normal(s) * 0.05)(D, F)), 'w_up': _w((lambda *s: _rng.normal(s) * 0.05)(D, F)), 'w_down': _w((lambda *s: _rng.normal(s) * 0.05)(F, D))}
    _B_in = _B_setup()
    return {'A_x': _A_in['x'], 'A_k_cache': _A_in['k_cache'], 'A_v_cache': _A_in['v_cache'], 'A_wq': _A_in['wq'], 'A_wo': _A_in['wo'], 'B_x': _B_in['x'], 'B_w_gate': _B_in['w_gate'], 'B_w_up': _B_in['w_up'], 'B_w_down': _B_in['w_down'], 'c': _w((lambda *s: _rng.normal(s) * 0.05)(8, 512)), 'w_mod': _w((lambda *s: _rng.normal(s) * 0.05)(512, 6 * 512) * 512 ** (-0.5))}

def reference(A_x, A_k_cache, A_v_cache, A_wq, A_wo, B_x, B_w_gate, B_w_up, B_w_down, c, w_mod):

    def _A_ref(x, k_cache, v_cache, wq, wo):
        B, Sq, D = x.shape
        Hq, Dh = (32, 128)
        Hkv, Sk = (k_cache.shape[1], k_cache.shape[2])
        W = min(4096, max(256, Sk // 4))
        rep = Hq // Hkv
        q = (lambda x, *d: x.transpose(*d))((x @ wq).reshape(B, Sq, Hq, Dh), 0, 2, 1, 3)
        k = jnp.repeat(k_cache[:, :, Sk - W:, :], rep, axis=1)
        v = jnp.repeat(v_cache[:, :, Sk - W:, :], rep, axis=1)
        scores = jnp.einsum('bhqd,bhkd->bhqk', q, k) * Dh ** (-0.5)
        p = _softmax(scores, axis=-1)
        o = jnp.einsum('bhqk,bhkd->bhqd', p, v)
        return (lambda x, *d: x.transpose(*d))(o, 0, 2, 1, 3).reshape(B, Sq, Hq * Dh) @ wo

    def _B_ref(x, w_gate, w_up, w_down):
        g = jnp.einsum('bsd,df->bsf', x, w_gate)
        u = jnp.einsum('bsd,df->bsf', x, w_up)
        h = _sigmoid(g) * u
        return jnp.einsum('bsf,fd->bsd', h, w_down)
    x = A_x
    mod = (_silu(c) @ w_mod).reshape(c.shape[0], 6, 1, -1)
    sa, ca, ga, sb, cb, gb = (mod[:, 0].copy(), mod[:, 1].copy(), mod[:, 2].copy(), mod[:, 3].copy(), mod[:, 4].copy(), mod[:, 5].copy())
    h = _layernorm(x, axis=-1) * (1 + ca) + sa
    x = x + ga * _A_ref(h, A_k_cache, A_v_cache, A_wq, A_wo)
    h = _layernorm(x, axis=-1) * (1 + cb) + sb
    x = x + gb * _B_ref(h, B_w_gate, B_w_up, B_w_down)
    return x
```

```python
import jax
import jax.numpy as jnp
from jax import lax
import jax.experimental.pallas as pl
import jax.experimental.pallas.tpu as pltpu

_B = 8
_D = 512
_H = 32
_DH = 128
_HG = 8
_NHG = _H // _HG
_NG = _B * _NHG
_PR = 16
_EPS = 1e-05

_NT = (((1,), (1,)), ((), ()))


def _layernorm(x):
    m = jnp.mean(x, axis=-1, keepdims=True)
    xc = x - m
    v = jnp.mean(xc * xc, axis=-1, keepdims=True)
    return xc / jnp.sqrt(v + _EPS)


def _make_kernel(sk, win, ffn):
    f32 = jnp.float32
    bf16 = jnp.bfloat16
    scale = _DH ** (-0.5)
    cw = _HG * _DH
    n_kv = win // _PR
    n_ffn = ffn // 32

    def kernel(x_hbm, k_hbm, v_hbm, wq_hbm, wo_hbm, wg_hbm, wu_hbm, wd_hbm, c_hbm, wm_hbm,
               o_ref,
               kbuf, vbuf, wq_buf, wo_buf, wg_buf, wu_buf, wd_buf, wm_buf, x_buf, c_buf,
               q_scr, o_scr, h_scr, acc_scr, kv_sem, sem):
        S_HEAD, S_WQ, S_WO, S_WM, S_GU, S_WD = range(6)

        def wait_all(buf, s):
            pltpu.make_async_copy(buf, buf, s).wait()

        def start_kv(g, slot):
            hg = g // _B
            b = g % _B
            h0 = pl.multiple_of(hg * _HG, _HG)
            for j in range(n_kv):
                pltpu.make_async_copy(
                    k_hbm.at[b, pl.ds(h0, _HG), pl.ds(sk - win + j * _PR, _PR), :],
                    kbuf.at[slot, :, pl.ds(j * _PR, _PR), :],
                    kv_sem.at[slot]).start(priority=0)
                pltpu.make_async_copy(
                    v_hbm.at[b, pl.ds(h0, _HG), pl.ds(sk - win + j * _PR, _PR), :],
                    vbuf.at[slot, :, pl.ds(j * _PR, _PR), :],
                    kv_sem.at[slot]).start(priority=1)

        def start_block(src, dst, r0, nr, c0, nc, s, prio):
            pltpu.make_async_copy(
                src.at[pl.ds(r0, nr), pl.ds(c0, nc)],
                dst.at[pl.ds(r0, nr), pl.ds(c0, nc)], s).start(priority=prio)

        pltpu.make_async_copy(c_hbm, c_buf, sem.at[S_HEAD]).start(priority=0)
        pltpu.make_async_copy(x_hbm, x_buf, sem.at[S_HEAD]).start(priority=1)
        for j in range(_D // 16):
            start_block(wm_hbm, wm_buf, j * 16, 16, 0, 2 * _D, sem.at[S_HEAD], j % 2)
        for j in range(_D // 16):
            start_block(wq_hbm, wq_buf, j * 16, 16, 0, cw, sem.at[S_WQ], j % 2)
        start_kv(0, 0)

        wait_all(c_buf, sem.at[S_HEAD])
        wait_all(x_buf, sem.at[S_HEAD])
        wait_all(wm_buf.at[:, pl.ds(0, 2 * _D)], sem.at[S_HEAD])
        cf = c_buf[...].astype(f32)
        sc = (cf * jax.nn.sigmoid(cf)).astype(bf16)
        mod_a = jnp.dot(sc, wm_buf[:, 0:2 * _D], preferred_element_type=f32)
        sa = mod_a[:, 0:_D]
        ca = mod_a[:, _D:2 * _D]
        x0 = x_buf[...].astype(f32)
        h_scr[...] = (_layernorm(x0) * (1.0 + ca) + sa).astype(bf16)
        acc_scr[...] = jnp.zeros((_B, _D), f32)

        def q_proj(hg):
            c0 = pl.multiple_of(hg * cw, cw)
            wait_all(wq_buf.at[:, pl.ds(0, cw)], sem.at[S_WQ])
            q = jnp.dot(h_scr[...], wq_buf[:, pl.ds(c0, cw)], preferred_element_type=f32)
            q = q.astype(bf16).astype(f32)
            for j in range(_HG):
                r0 = pl.multiple_of((hg * _HG + j) * _B, _B)
                q_scr[pl.ds(r0, _B), :] = q[:, j * _DH:(j + 1) * _DH]

        q_proj(0)

        row_s = lax.broadcasted_iota(jnp.int32, (_HG, win), 0)
        row_o = lax.broadcasted_iota(jnp.int32, (_HG, _DH), 0)

        def body(g, carry):
            slot = g % 2
            hg = g // _B
            b = g % _B

            r_wo = pl.multiple_of(g * _DH, _DH)
            for j in range(4):
                start_block(wo_hbm, wo_buf, r_wo + j * 32, 32, 0, _D, sem.at[S_WO], j % 2)
            r_wm = pl.multiple_of(g * 16, 16)
            for j in range(2):
                start_block(wm_hbm, wm_buf, r_wm, 16, 2 * _D + j * 2 * _D, 2 * _D, sem.at[S_WM], j % 2)

            @pl.when(hg < _NHG - 1)
            def _():
                r_wq = pl.multiple_of(b * 64, 64)
                c_wq = pl.multiple_of((hg + 1) * cw, cw)
                for j in range(4):
                    start_block(wq_hbm, wq_buf, r_wq + j * 16, 16, c_wq, cw, sem.at[S_WQ], j % 2)

            @pl.when(g + 1 < _NG)
            def _():
                start_kv(g + 1, 1 - slot)

            @pl.when(g + 1 == _NG)
            def _():
                for j in range(n_ffn):
                    start_block(wg_hbm, wg_buf, j * 32, 32, 0, _D, sem.at[S_GU], 0)
                    start_block(wu_hbm, wu_buf, j * 32, 32, 0, _D, sem.at[S_GU], 1)
                for j in range(n_ffn):
                    start_block(wd_hbm, wd_buf, j * 32, 32, 0, _D, sem.at[S_WD], j % 2)

            wait_all(kbuf.at[slot], kv_sem.at[slot])
            wait_all(vbuf.at[slot], kv_sem.at[slot])

            qrow = hg * (_HG * _B) + b
            q8 = q_scr[pl.ds(qrow, _HG, stride=_B), :].astype(bf16)
            s_all = jnp.zeros((_HG, win), f32)
            for j in range(_HG):
                s = lax.dot_general(q8, kbuf[slot, j], _NT, preferred_element_type=f32)
                s_all = jnp.where(row_s == j, s, s_all)
            s_all = s_all * scale
            m = jnp.max(s_all, axis=-1, keepdims=True)
            p = jnp.exp(s_all - m)
            l = jnp.sum(p, axis=-1, keepdims=True)
            pb = p.astype(bf16)
            o_all = jnp.zeros((_HG, _DH), f32)
            for j in range(_HG):
                o = jnp.dot(pb, vbuf[slot, j], preferred_element_type=f32)
                o_all = jnp.where(row_o == j, o, o_all)
            o_scr[pl.ds(b, _HG, stride=_B), :] = o_all / l

            @pl.when(b == _B - 1)
            def _():
                wait_all(wo_buf.at[pl.ds(0, cw), :], sem.at[S_WO])
                oc = jnp.concatenate(
                    [o_scr[j * _B:(j + 1) * _B, :] for j in range(_HG)], axis=-1).astype(bf16)
                r0 = pl.multiple_of(hg * cw, cw)
                acc_scr[...] += jnp.dot(oc, wo_buf[pl.ds(r0, cw), :], preferred_element_type=f32)

                @pl.when(hg < _NHG - 1)
                def _():
                    q_proj(hg + 1)

            return carry

        lax.fori_loop(0, _NG, body, 0)

        wait_all(wm_buf.at[:, pl.ds(2 * _D, 4 * _D)], sem.at[S_WM])
        mod_b = jnp.dot(sc, wm_buf[:, 2 * _D:6 * _D], preferred_element_type=f32)
        ga = mod_b[:, 0:_D]
        sb = mod_b[:, _D:2 * _D]
        cb = mod_b[:, 2 * _D:3 * _D]
        gb = mod_b[:, 3 * _D:4 * _D]
        x1 = x0 + ga * acc_scr[...]
        h2 = (_layernorm(x1) * (1.0 + cb) + sb).astype(bf16)
        wait_all(wg_buf, sem.at[S_GU])
        wait_all(wu_buf, sem.at[S_GU])
        gt = lax.dot_general(h2, wg_buf[...], _NT, preferred_element_type=f32)
        up = lax.dot_general(h2, wu_buf[...], _NT, preferred_element_type=f32)
        act = (jax.nn.sigmoid(gt) * up).astype(bf16)
        wait_all(wd_buf, sem.at[S_WD])
        y = jnp.dot(act, wd_buf[...], preferred_element_type=f32)
        o_ref[...] = (x1 + gb * y).astype(o_ref.dtype)

    return kernel


@jax.jit
def pallas_adaLN_cond__sliding_block_cached__glu_gated_glu__decode_kernel(
    A_x: jax.Array,
    A_k_cache: jax.Array,
    A_v_cache: jax.Array,
    A_wq: jax.Array,
    A_wo: jax.Array,
    B_x: jax.Array,
    B_w_gate: jax.Array,
    B_w_up: jax.Array,
    B_w_down: jax.Array,
    c: jax.Array,
    w_mod: jax.Array,
):
    del B_x
    sk = A_k_cache.shape[2]
    win = min(4096, max(256, sk // 4))
    ffn = B_w_down.shape[0]
    bf16 = jnp.bfloat16
    f32 = jnp.float32

    hbm = pl.BlockSpec(memory_space=pltpu.MemorySpace.HBM)
    out = pl.pallas_call(
        _make_kernel(sk, win, ffn),
        in_specs=[hbm] * 10,
        out_specs=pl.BlockSpec(memory_space=pltpu.MemorySpace.VMEM),
        out_shape=jax.ShapeDtypeStruct((_B, _D), A_x.dtype),
        scratch_shapes=[
            pltpu.VMEM((2, _HG, win, _DH), bf16),
            pltpu.VMEM((2, _HG, win, _DH), bf16),
            pltpu.VMEM((_D, _H * _DH), bf16),
            pltpu.VMEM((_H * _DH, _D), bf16),
            pltpu.VMEM((ffn, _D), bf16),
            pltpu.VMEM((ffn, _D), bf16),
            pltpu.VMEM((ffn, _D), bf16),
            pltpu.VMEM((_D, 6 * _D), bf16),
            pltpu.VMEM((_B, _D), bf16),
            pltpu.VMEM((_B, _D), bf16),
            pltpu.VMEM((_H * _B, _DH), f32),
            pltpu.VMEM((_HG * _B, _DH), f32),
            pltpu.VMEM((_B, _D), bf16),
            pltpu.VMEM((_B, _D), f32),
            pltpu.SemaphoreType.DMA((2,)),
            pltpu.SemaphoreType.DMA((6,)),
        ],
        compiler_params=pltpu.CompilerParams(vmem_limit_bytes=64 * 1024 * 1024),
    )(A_x.reshape(_B, _D), A_k_cache, A_v_cache, A_wq, A_wo,
      B_w_gate.T, B_w_up.T, B_w_down, c, w_mod)
    return out.reshape(A_x.shape)
```

```python
import jax
import jax.numpy as jnp
from jax import lax
import jax.experimental.pallas as pl
import jax.experimental.pallas.tpu as pltpu

_B = 8
_D = 512
_H = 32
_DH = 128
_HU = 16
_NI = _B * _H // _HU
_PR = 16
_EPS = 1e-05
_LAG = 26
_GU_HEAD = 24

_NT = (((1,), (1,)), ((), ()))


def _layernorm(x):
    m = jnp.mean(x, axis=-1, keepdims=True)
    xc = x - m
    v = jnp.mean(xc * xc, axis=-1, keepdims=True)
    return xc / jnp.sqrt(v + _EPS)


def _merge(*lists):
    keyed = []
    for k, lst in enumerate(lists):
        keyed += [((j + 0.5) / len(lst), k, j) for j in range(len(lst))]
    return [lists[k][j] for _, k, j in sorted(keyed)]


def _make_kernel(sk, win, ffn):
    f32 = jnp.float32
    bf16 = jnp.bfloat16
    scale = _DH ** (-0.5)
    cw = _HU * _DH
    n_kv = win // _PR
    n_ffn = ffn // 32
    gu_bounds = (0, _GU_HEAD * 32, ffn)
    d_bounds = (0, 896, 1152, ffn)
    s_k, s_v, s_mod, s_wq, s_wo, s_gu = 0, 2, 4, 5, 6, 7
    s_wd = s_gu + len(gu_bounds) - 1
    n_sem = s_wd + len(d_bounds) - 1

    def kernel(x_hbm, k_hbm, v_hbm, wq_hbm, wo_hbm, wg_hbm, wu_hbm, wd_hbm, c_hbm, wm_hbm,
               o_ref,
               kbuf, vbuf, wq_buf, wo_buf, wg_buf, wu_buf, wd_buf, wm_buf, x_buf, c_buf,
               q_scr, o_scr, h_scr, acc_scr, mod_scr, act_scr, p_scr, l_scr, sem):

        def start(cp, thread):
            pltpu.make_async_copy(cp[0], cp[1], sem.at[cp[2]]).start(priority=thread)

        def start_pairs(his, los):
            for j in range(max(len(his), len(los))):
                if j < len(his):
                    start(his[j], 0)
                if j < len(los):
                    start(los[j], 1)

        def wait_filled(region, s):
            pltpu.make_async_copy(region, region, sem.at[s]).wait()

        def kv_list(i, w, thread, j0, j1):
            slot = i % 2
            h0 = (i // _B) * _HU + thread * 8
            heads = pl.ds(h0 if isinstance(h0, int) else pl.multiple_of(h0, 8), 8)
            src, dst, s = ((k_hbm, kbuf, s_k), (v_hbm, vbuf, s_v))[w]
            return [(src.at[i % _B, heads, pl.ds(sk - win + j * _PR, _PR), :],
                     dst.at[slot, pl.ds(thread * 8, 8), pl.ds(j * _PR, _PR), :], s + slot)
                    for j in range(j0, j1)]

        def rows32(src, dst, j, s):
            return (src.at[pl.ds(j * 32, 32), :], dst.at[pl.ds(j * 32, 32), :], s)

        def quads(src, dst, s):
            return [(src.at[:, pl.ds(r, 8), pl.ds(c, 512)], dst.at[:, pl.ds(r, 8), pl.ds(c, 512)], s)
                    for r in range(0, src.shape[1], 8) for c in range(0, src.shape[2], 512)]

        def gate_up(j0, j1, s):
            out = []
            for j in range(j0, j1):
                out += [rows32(wg_hbm, wg_buf, j, s), rows32(wu_hbm, wu_buf, j, s)]
            return out

        def tail_lists():
            gu = gate_up(_GU_HEAD, n_ffn, s_gu + 1)
            dn = [rows32(wd_hbm, wd_buf, j, s_wd + sum(j * 32 >= r for r in d_bounds[1:]))
                  for j in range(n_ffn)]
            n_lo_gu = (len(gu) + len(dn) + _LAG) // 2 - len(dn)
            return gu[n_lo_gu:], gu[:n_lo_gu] + dn

        def issue_unit(i, w, next_lo):
            start_pairs(kv_list(i, w, 0, 0, n_kv), kv_list(i, w, 1, _LAG, n_kv) + next_lo)

        head = [(c_hbm, c_buf, s_mod), (x_hbm, x_buf, s_mod)]
        head += _merge(quads(wm_hbm, wm_buf, s_mod), gate_up(0, _GU_HEAD, s_gu))
        head += _merge(quads(wq_hbm, wq_buf, s_wq), quads(wo_hbm, wo_buf, s_wo))
        head_hi, head_lo = head[0::2], head[1::2]
        start_pairs([], head_lo[:_LAG])
        start_pairs(head_hi, head_lo[_LAG:] + kv_list(0, 0, 1, 0, _LAG))
        issue_unit(0, 0, kv_list(0, 1, 1, 0, _LAG))

        wait_filled(c_buf, s_mod)
        wait_filled(x_buf, s_mod)
        wait_filled(wm_buf, s_mod)

        def mod_cols(c0, c1):
            cf = c_buf[...].astype(f32)
            silu_c = (cf * jax.nn.sigmoid(cf)).astype(bf16)
            w = wm_buf[:, :, c0:c1].reshape(_D, c1 - c0)
            return jnp.dot(silu_c, w, preferred_element_type=f32)

        mod_a = mod_cols(0, 2 * _D)
        shift_a = mod_a[:, 0:_D]
        scale_a = mod_a[:, _D:2 * _D]
        h_scr[...] = (_layernorm(x_buf[...].astype(f32)) * (1.0 + scale_a) + shift_a).astype(bf16)

        def q_proj(half):
            w = wq_buf[:, :, half * cw:(half + 1) * cw].reshape(_D, cw)
            q = jnp.dot(h_scr[...], w, preferred_element_type=f32).astype(bf16).astype(f32)
            for j in range(_HU):
                r0 = (half * _HU + j) * _B
                q_scr[r0:r0 + _B, :] = q[:, j * _DH:(j + 1) * _DH]

        def o_proj(half):
            r0 = half * _HU * _B
            oc = jnp.concatenate(
                [o_scr[r0 + j * _B:r0 + (j + 1) * _B, :] for j in range(_HU)], axis=-1)
            w = wo_buf[2 * half:2 * half + 2].reshape(cw, _D)
            return jnp.dot(oc.astype(bf16), w, preferred_element_type=f32)

        wait_filled(wq_buf, s_wq)
        wait_filled(wo_buf, s_wo)
        q_proj(0)

        row_s = lax.broadcasted_iota(jnp.int32, (8, win), 0)
        row_o = lax.broadcasted_iota(jnp.int32, (8, _DH), 0)

        def body(i, carry):
            slot = i % 2
            rows8 = [pl.ds(((i // _B) * _HU + t * 8) * _B + i % _B, 8, stride=_B) for t in range(2)]

            @pl.when(i + 1 < _NI)
            def _():
                issue_unit(i, 1, kv_list(i + 1, 0, 1, 0, _LAG))

            @pl.when(i + 1 == _NI)
            def _():
                issue_unit(_NI - 1, 1, tail_lists()[1][:_LAG])

            wait_filled(kbuf.at[slot], s_k + slot)
            for t in range(2):
                q8 = q_scr[rows8[t], :].astype(bf16)
                s_all = jnp.zeros((8, win), f32)
                for j in range(8):
                    s = lax.dot_general(q8, kbuf[slot, t * 8 + j], _NT, preferred_element_type=f32)
                    s_all = jnp.where(row_s == j, s, s_all)
                s_all = s_all * scale
                m = jnp.max(s_all, axis=-1, keepdims=True)
                p = jnp.exp(s_all - m)
                l_scr[t] = jnp.broadcast_to(jnp.sum(p, axis=-1, keepdims=True), (8, _DH))
                p_scr[t] = p

            @pl.when(i + 1 < _NI)
            def _():
                issue_unit(i + 1, 0, kv_list(i + 1, 1, 1, 0, _LAG))

            @pl.when(i + 1 == _NI)
            def _():
                tail_hi, tail_lo = tail_lists()
                start_pairs(tail_hi, tail_lo[_LAG:])

            wait_filled(vbuf.at[slot], s_v + slot)
            for t in range(2):
                pb = p_scr[t].astype(bf16)
                o_all = jnp.zeros((8, _DH), f32)
                for j in range(8):
                    o = jnp.dot(pb, vbuf[slot, t * 8 + j], preferred_element_type=f32)
                    o_all = jnp.where(row_o == j, o, o_all)
                o_scr[rows8[t], :] = o_all / l_scr[t]

            @pl.when(i == 1)
            def _():
                mod_scr[...] = mod_cols(2 * _D, 6 * _D)

            @pl.when(i == 2)
            def _():
                q_proj(1)

            @pl.when(i == _B)
            def _():
                acc_scr[...] = o_proj(0)

            return carry

        lax.fori_loop(0, _NI, body, 0)

        gate_a = mod_scr[:, 0:_D]
        shift_b = mod_scr[:, _D:2 * _D]
        scale_b = mod_scr[:, 2 * _D:3 * _D]
        gate_b = mod_scr[:, 3 * _D:4 * _D]
        x1 = x_buf[...].astype(f32) + gate_a * (acc_scr[...] + o_proj(1))
        h2 = (_layernorm(x1) * (1.0 + scale_b) + shift_b).astype(bf16)
        for n in range(len(gu_bounds) - 1):
            r0, r1 = gu_bounds[n], gu_bounds[n + 1]
            wait_filled(wg_buf.at[r0:r1, :], s_gu + n)
            wait_filled(wu_buf.at[r0:r1, :], s_gu + n)
            gt = lax.dot_general(h2, wg_buf[r0:r1, :], _NT, preferred_element_type=f32)
            up = lax.dot_general(h2, wu_buf[r0:r1, :], _NT, preferred_element_type=f32)
            act_scr[:, r0:r1] = jax.nn.sigmoid(gt) * up
        for n in range(len(d_bounds) - 1):
            r0, r1 = d_bounds[n], d_bounds[n + 1]
            wait_filled(wd_buf.at[r0:r1, :], s_wd + n)
            y = jnp.dot(act_scr[:, r0:r1].astype(bf16), wd_buf[r0:r1, :], preferred_element_type=f32)
            if n == 0:
                acc_scr[...] = x1 + gate_b * y
            elif n < len(d_bounds) - 2:
                acc_scr[...] += gate_b * y
            else:
                o_ref[...] = (acc_scr[...] + gate_b * y).astype(o_ref.dtype)

    return kernel, n_sem


@jax.jit
def pallas_adaLN_cond__sliding_block_cached__glu_gated_glu__decode_kernel(
    A_x: jax.Array,
    A_k_cache: jax.Array,
    A_v_cache: jax.Array,
    A_wq: jax.Array,
    A_wo: jax.Array,
    B_x: jax.Array,
    B_w_gate: jax.Array,
    B_w_up: jax.Array,
    B_w_down: jax.Array,
    c: jax.Array,
    w_mod: jax.Array,
):
    del B_x
    sk = A_k_cache.shape[2]
    win = min(4096, max(256, sk // 4))
    ffn = B_w_down.shape[0]
    assert A_x.shape == (_B, 1, _D) and A_k_cache.shape == (_B, _H, sk, _DH)
    assert win == 1024 and ffn == 1376
    bf16 = jnp.bfloat16
    f32 = jnp.float32
    kernel, n_sem = _make_kernel(sk, win, ffn)

    hbm = pl.BlockSpec(memory_space=pltpu.MemorySpace.HBM)
    out = pl.pallas_call(
        kernel,
        in_specs=[hbm] * 10,
        out_specs=pl.BlockSpec(memory_space=pltpu.MemorySpace.VMEM),
        out_shape=jax.ShapeDtypeStruct((_B, _D), A_x.dtype),
        scratch_shapes=[
            pltpu.VMEM((2, _HU, win, _DH), bf16),
            pltpu.VMEM((2, _HU, win, _DH), bf16),
            pltpu.VMEM((4, _D // 4, _H * _DH), bf16),
            pltpu.VMEM((4, _H * _DH // 4, _D), bf16),
            pltpu.VMEM((ffn, _D), bf16),
            pltpu.VMEM((ffn, _D), bf16),
            pltpu.VMEM((ffn, _D), bf16),
            pltpu.VMEM((4, _D // 4, 6 * _D), bf16),
            pltpu.VMEM((_B, _D), bf16),
            pltpu.VMEM((_B, _D), bf16),
            pltpu.VMEM((_H * _B, _DH), f32),
            pltpu.VMEM((_H * _B, _DH), f32),
            pltpu.VMEM((_B, _D), bf16),
            pltpu.VMEM((_B, _D), f32),
            pltpu.VMEM((_B, 4 * _D), f32),
            pltpu.VMEM((_B, ffn), f32),
            pltpu.VMEM((2, 8, win), f32),
            pltpu.VMEM((2, 8, _DH), f32),
            pltpu.SemaphoreType.DMA((n_sem,)),
        ],
        compiler_params=pltpu.CompilerParams(
            vmem_limit_bytes=64 * 1024 * 1024,
            disable_bounds_checks=True,
            disable_semaphore_checks=True,
        ),
    )(
        A_x.reshape(_B, _D),
        A_k_cache,
        A_v_cache,
        A_wq.reshape(4, _D // 4, _H * _DH),
        A_wo.reshape(4, _H * _DH // 4, _D),
        B_w_gate.T,
        B_w_up.T,
        B_w_down,
        c,
        w_mod.reshape(4, _D // 4, 6 * _D),
    )
    return out.reshape(A_x.shape)
```

```python
import jax
import jax.numpy as jnp
from jax import lax
import jax.experimental.pallas as pl
import jax.experimental.pallas.tpu as pltpu

_B = 8
_D = 512
_H = 32
_DH = 128
_HU = 16
_NI = _B * _H // _HU
_PR = 16
_EPS = 1e-05
_LAG = 26
_GU_HEAD = 24

_NT = (((1,), (1,)), ((), ()))


def _layernorm(x):
    m = jnp.mean(x, axis=-1, keepdims=True)
    xc = x - m
    v = jnp.mean(xc * xc, axis=-1, keepdims=True)
    return xc / jnp.sqrt(v + _EPS)


def _merge(*lists):
    keyed = []
    for k, lst in enumerate(lists):
        keyed += [((j + 0.5) / len(lst), k, j) for j in range(len(lst))]
    return [lists[k][j] for _, k, j in sorted(keyed)]


def _make_kernel(sk, win, ffn):
    f32 = jnp.float32
    bf16 = jnp.bfloat16
    scale = _DH ** (-0.5)
    cw = _HU * _DH
    n_kv = win // _PR
    n_ffn = ffn // 32
    gu_bounds = (0, _GU_HEAD * 32, ffn)
    d_bounds = (0, 896, 1152, ffn)
    s_k, s_v, s_c, s_x, s_wm, s_wq, s_wo, s_wg = 0, 2, 4, 5, 6, 7, 8, 9
    s_wu = s_wg + len(gu_bounds) - 1
    s_wd = s_wu + len(gu_bounds) - 1
    n_sem = s_wd + len(d_bounds) - 1

    def kernel(x_hbm, k_hbm, v_hbm, wq_hbm, wo_hbm, wg_hbm, wu_hbm, wd_hbm, c_hbm, wm_hbm,
               o_ref,
               kbuf, vbuf, wq_buf, wo_buf, wg_buf, wu_buf, wd_buf, wm_buf, x_buf, c_buf,
               q_scr, o_scr, h_scr, acc_scr, mod_scr, act_scr, p_scr, l_scr, sem):

        def start(cp, thread):
            pltpu.make_async_copy(cp[0], cp[1], sem.at[cp[2]]).start(priority=thread)

        def start_pairs(his, los):
            for j in range(max(len(his), len(los))):
                if j < len(his):
                    start(his[j], 0)
                if j < len(los):
                    start(los[j], 1)

        def wait_filled(region, s):
            pltpu.make_async_copy(region, region, sem.at[s]).wait()

        def kv_list(i, w, thread, j0, j1):
            slot = i % 2
            h0 = (i // _B) * _HU + thread * 8
            heads = pl.ds(h0 if isinstance(h0, int) else pl.multiple_of(h0, 8), 8)
            src, dst, s = ((k_hbm, kbuf, s_k), (v_hbm, vbuf, s_v))[w]
            return [(src.at[i % _B, heads, pl.ds(sk - win + j * _PR, _PR), :],
                     dst.at[slot, pl.ds(thread * 8, 8), pl.ds(j * _PR, _PR), :], s + slot)
                    for j in range(j0, j1)]

        def rows32(src, dst, j, s):
            return (src.at[pl.ds(j * 32, 32), :], dst.at[pl.ds(j * 32, 32), :], s)

        def quads(src, dst, s):
            return [(src.at[:, pl.ds(r, 8), pl.ds(c, 512)], dst.at[:, pl.ds(r, 8), pl.ds(c, 512)], s)
                    for r in range(0, src.shape[1], 8) for c in range(0, src.shape[2], 512)]

        def gate_up(j0, j1, n):
            out = []
            for j in range(j0, j1):
                out += [rows32(wg_hbm, wg_buf, j, s_wg + n), rows32(wu_hbm, wu_buf, j, s_wu + n)]
            return out

        def tail_lists():
            gu = gate_up(_GU_HEAD, n_ffn, 1)
            dn = [rows32(wd_hbm, wd_buf, j, s_wd + sum(j * 32 >= r for r in d_bounds[1:]))
                  for j in range(n_ffn)]
            n_lo_gu = (len(gu) + len(dn) + _LAG) // 2 - len(dn)
            return gu[n_lo_gu:], gu[:n_lo_gu] + dn

        def issue_unit(i, w, next_lo):
            start_pairs(kv_list(i, w, 0, 0, n_kv), kv_list(i, w, 1, _LAG, n_kv) + next_lo)

        head = [(c_hbm, c_buf, s_c), (x_hbm, x_buf, s_x)]
        head += _merge(quads(wm_hbm, wm_buf, s_wm), gate_up(0, _GU_HEAD, 0))
        head += _merge(quads(wq_hbm, wq_buf, s_wq), quads(wo_hbm, wo_buf, s_wo))
        head_hi, head_lo = head[0::2], head[1::2]
        start_pairs([], head_lo[:_LAG])
        start_pairs(head_hi, head_lo[_LAG:] + kv_list(0, 0, 1, 0, _LAG))
        issue_unit(0, 0, kv_list(0, 1, 1, 0, _LAG))

        wait_filled(c_buf, s_c)
        wait_filled(x_buf, s_x)
        wait_filled(wm_buf, s_wm)

        def mod_cols(c0, c1):
            cf = c_buf[...].astype(f32)
            silu_c = (cf * jax.nn.sigmoid(cf)).astype(bf16)
            w = wm_buf[:, :, c0:c1].reshape(_D, c1 - c0)
            return jnp.dot(silu_c, w, preferred_element_type=f32)

        mod_a = mod_cols(0, 2 * _D)
        shift_a = mod_a[:, 0:_D]
        scale_a = mod_a[:, _D:2 * _D]
        h_scr[...] = (_layernorm(x_buf[...].astype(f32)) * (1.0 + scale_a) + shift_a).astype(bf16)

        def q_proj(half):
            w = wq_buf[:, :, half * cw:(half + 1) * cw].reshape(_D, cw)
            q = jnp.dot(h_scr[...], w, preferred_element_type=f32).astype(bf16).astype(f32)
            for j in range(_HU):
                r0 = (half * _HU + j) * _B
                q_scr[r0:r0 + _B, :] = q[:, j * _DH:(j + 1) * _DH]

        def o_proj(half):
            r0 = half * _HU * _B
            oc = jnp.concatenate(
                [o_scr[r0 + j * _B:r0 + (j + 1) * _B, :] for j in range(_HU)], axis=-1)
            w = wo_buf[2 * half:2 * half + 2].reshape(cw, _D)
            return jnp.dot(oc.astype(bf16), w, preferred_element_type=f32)

        wait_filled(wq_buf, s_wq)
        wait_filled(wo_buf, s_wo)
        q_proj(0)

        row_s = lax.broadcasted_iota(jnp.int32, (8, win), 0)
        row_o = lax.broadcasted_iota(jnp.int32, (8, _DH), 0)

        def body(i, carry):
            slot = i % 2
            rows8 = [pl.ds(((i // _B) * _HU + t * 8) * _B + i % _B, 8, stride=_B) for t in range(2)]

            @pl.when(i + 1 < _NI)
            def _():
                issue_unit(i, 1, kv_list(i + 1, 0, 1, 0, _LAG))

            @pl.when(i + 1 == _NI)
            def _():
                issue_unit(_NI - 1, 1, tail_lists()[1][:_LAG])

            wait_filled(kbuf.at[slot], s_k + slot)
            for t in range(2):
                q8 = q_scr[rows8[t], :].astype(bf16)
                s_all = jnp.zeros((8, win), f32)
                for j in range(8):
                    s = lax.dot_general(q8, kbuf[slot, t * 8 + j], _NT, preferred_element_type=f32)
                    s_all = jnp.where(row_s == j, s, s_all)
                s_all = s_all * scale
                m = jnp.max(s_all, axis=-1, keepdims=True)
                p = jnp.exp(s_all - m)
                l_scr[t] = jnp.broadcast_to(jnp.sum(p, axis=-1, keepdims=True), (8, _DH))
                p_scr[t] = p

            @pl.when(i + 1 < _NI)
            def _():
                issue_unit(i + 1, 0, kv_list(i + 1, 1, 1, 0, _LAG))

            @pl.when(i + 1 == _NI)
            def _():
                tail_hi, tail_lo = tail_lists()
                start_pairs(tail_hi, tail_lo[_LAG:])

            wait_filled(vbuf.at[slot], s_v + slot)
            for t in range(2):
                pb = p_scr[t].astype(bf16)
                o_all = jnp.zeros((8, _DH), f32)
                for j in range(8):
                    o = jnp.dot(pb, vbuf[slot, t * 8 + j], preferred_element_type=f32)
                    o_all = jnp.where(row_o == j, o, o_all)
                o_scr[rows8[t], :] = o_all / l_scr[t]

            @pl.when(i == 1)
            def _():
                mod_scr[...] = mod_cols(2 * _D, 6 * _D)

            @pl.when(i == 2)
            def _():
                q_proj(1)

            @pl.when(i == _B)
            def _():
                acc_scr[...] = o_proj(0)

            return carry

        lax.fori_loop(0, _NI, body, 0)

        gate_a = mod_scr[:, 0:_D]
        shift_b = mod_scr[:, _D:2 * _D]
        scale_b = mod_scr[:, 2 * _D:3 * _D]
        gate_b = mod_scr[:, 3 * _D:4 * _D]
        x1 = x_buf[...].astype(f32) + gate_a * (acc_scr[...] + o_proj(1))
        h2 = (_layernorm(x1) * (1.0 + scale_b) + shift_b).astype(bf16)
        for n in range(len(gu_bounds) - 1):
            r0, r1 = gu_bounds[n], gu_bounds[n + 1]
            wait_filled(wg_buf.at[r0:r1, :], s_wg + n)
            wait_filled(wu_buf.at[r0:r1, :], s_wu + n)
            gt = lax.dot_general(h2, wg_buf[r0:r1, :], _NT, preferred_element_type=f32)
            up = lax.dot_general(h2, wu_buf[r0:r1, :], _NT, preferred_element_type=f32)
            act_scr[:, r0:r1] = jax.nn.sigmoid(gt) * up
        for n in range(len(d_bounds) - 1):
            r0, r1 = d_bounds[n], d_bounds[n + 1]
            wait_filled(wd_buf.at[r0:r1, :], s_wd + n)
            y = jnp.dot(act_scr[:, r0:r1].astype(bf16), wd_buf[r0:r1, :], preferred_element_type=f32)
            if n == 0:
                acc_scr[...] = x1 + gate_b * y
            elif n < len(d_bounds) - 2:
                acc_scr[...] += gate_b * y
            else:
                o_ref[...] = (acc_scr[...] + gate_b * y).astype(o_ref.dtype)

    return kernel, n_sem


@jax.jit
def pallas_adaLN_cond__sliding_block_cached__glu_gated_glu__decode_kernel(
    A_x: jax.Array,
    A_k_cache: jax.Array,
    A_v_cache: jax.Array,
    A_wq: jax.Array,
    A_wo: jax.Array,
    B_x: jax.Array,
    B_w_gate: jax.Array,
    B_w_up: jax.Array,
    B_w_down: jax.Array,
    c: jax.Array,
    w_mod: jax.Array,
):
    del B_x
    sk = A_k_cache.shape[2]
    win = min(4096, max(256, sk // 4))
    ffn = B_w_down.shape[0]
    assert A_x.shape == (_B, 1, _D) and A_k_cache.shape == (_B, _H, sk, _DH)
    assert win == 1024 and ffn == 1376
    bf16 = jnp.bfloat16
    f32 = jnp.float32
    kernel, n_sem = _make_kernel(sk, win, ffn)

    hbm = pl.BlockSpec(memory_space=pltpu.MemorySpace.HBM)
    out = pl.pallas_call(
        kernel,
        in_specs=[hbm] * 10,
        out_specs=pl.BlockSpec(memory_space=pltpu.MemorySpace.VMEM),
        out_shape=jax.ShapeDtypeStruct((_B, _D), A_x.dtype),
        scratch_shapes=[
            pltpu.VMEM((2, _HU, win, _DH), bf16),
            pltpu.VMEM((2, _HU, win, _DH), bf16),
            pltpu.VMEM((4, _D // 4, _H * _DH), bf16),
            pltpu.VMEM((4, _H * _DH // 4, _D), bf16),
            pltpu.VMEM((ffn, _D), bf16),
            pltpu.VMEM((ffn, _D), bf16),
            pltpu.VMEM((ffn, _D), bf16),
            pltpu.VMEM((4, _D // 4, 6 * _D), bf16),
            pltpu.VMEM((_B, _D), bf16),
            pltpu.VMEM((_B, _D), bf16),
            pltpu.VMEM((_H * _B, _DH), f32),
            pltpu.VMEM((_H * _B, _DH), f32),
            pltpu.VMEM((_B, _D), bf16),
            pltpu.VMEM((_B, _D), f32),
            pltpu.VMEM((_B, 4 * _D), f32),
            pltpu.VMEM((_B, ffn), f32),
            pltpu.VMEM((2, 8, win), f32),
            pltpu.VMEM((2, 8, _DH), f32),
            pltpu.SemaphoreType.DMA((n_sem,)),
        ],
        compiler_params=pltpu.CompilerParams(
            vmem_limit_bytes=64 * 1024 * 1024,
            disable_bounds_checks=True,
            disable_semaphore_checks=True,
        ),
    )(
        A_x.reshape(_B, _D),
        A_k_cache,
        A_v_cache,
        A_wq.reshape(4, _D // 4, _H * _DH),
        A_wo.reshape(4, _H * _DH // 4, _D),
        B_w_gate.T,
        B_w_up.T,
        B_w_down,
        c,
        w_mod.reshape(4, _D // 4, 6 * _D),
    )
    return out.reshape(A_x.shape)
```

```python
import jax
import jax.numpy as jnp
from jax import lax
import jax.experimental.pallas as pl
import jax.experimental.pallas.tpu as pltpu

_B = 8
_D = 512
_H = 32
_DH = 128
_NW = _B * _H
_HU = 16
_NI = _NW // _HU
_PR = 16
_OFF = 2
_EPS = 1e-05
_LAG = 26
_GU_HEAD = 24

_NT = (((1,), (1,)), ((), ()))


def _layernorm(x):
    m = jnp.mean(x, axis=-1, keepdims=True)
    xc = x - m
    v = jnp.mean(xc * xc, axis=-1, keepdims=True)
    return xc / jnp.sqrt(v + _EPS)


def _merge(*lists):
    keyed = []
    for k, lst in enumerate(lists):
        keyed += [((j + 0.5) / len(lst), k, j) for j in range(len(lst))]
    return [lists[k][j] for _, k, j in sorted(keyed)]


def _make_kernel(sk, win, ffn):
    f32 = jnp.float32
    bf16 = jnp.bfloat16
    scale = _DH ** (-0.5)
    pad = 8 - _OFF
    n_kv = win // _PR
    n_ffn = ffn // 32
    gu_bounds = (0, _GU_HEAD * 32, ffn)
    d_bounds = (0, 896, 1152, ffn)
    s_k, s_v, s_c, s_x, s_wm, s_wq, s_wo, s_wg = 0, 2, 4, 5, 6, 7, 8, 9
    s_wu = s_wg + len(gu_bounds) - 1
    s_wd = s_wu + len(gu_bounds) - 1
    n_sem = s_wd + len(d_bounds) - 1

    def kernel(x_hbm, k_hbm, v_hbm, wq_hbm, wo_hbm, wg_hbm, wu_hbm, wd_hbm, c_hbm, wm_hbm,
               o_ref,
               kbuf, vbuf, wq_buf, wo_buf, wg_buf, wu_buf, wd_buf, wm_buf, x_buf, c_buf,
               q_scr, o_scr, h_scr, acc_scr, mod_scr, act_scr, p_scr, l_scr, sem):

        def start(cp, thread):
            for src, dst, s in (cp if isinstance(cp, list) else [cp]):
                pltpu.make_async_copy(src, dst, sem.at[s]).start(priority=thread)

        def start_pairs(his, los):
            for j in range(max(len(his), len(los))):
                if j < len(his):
                    start(his[j], 0)
                if j < len(los):
                    start(los[j], 1)

        def wait_filled(region, s):
            pltpu.make_async_copy(region, region, sem.at[s]).wait()

        def block_of(i, t):
            return 4 * (i % _B) + (1 - i // _B if t == 0 else 2 + i // _B)

        def kv_list(i, w, thread, j0, j1):
            slot = i % 2
            t = 1 - thread
            w0 = _OFF + 8 * block_of(i, t)
            src, dst, s = ((k_hbm, kbuf, s_k), (v_hbm, vbuf, s_v))[w]
            parts = [(w0, 8 * t, 8)]
            if isinstance(w0, int) and w0 + 8 > _NW:
                parts = [(w0, 8 * t, _NW - w0), (0, 8 * t + _NW - w0, w0 + 8 - _NW)]
            return [[(src.at[pl.ds(ws, n), pl.ds(sk - win + j * _PR, _PR), :],
                      dst.at[slot, pl.ds(wd, n), pl.ds(j * _PR, _PR), :], s + slot)
                     for ws, wd, n in parts] for j in range(j0, j1)]

        def rows32(src, dst, j, s):
            return (src.at[pl.ds(j * 32, 32), :], dst.at[pl.ds(j * 32, 32), :], s)

        def quads(src, dst, s):
            return [(src.at[:, pl.ds(r, 8), pl.ds(c, 512)], dst.at[:, pl.ds(r, 8), pl.ds(c, 512)], s)
                    for r in range(0, src.shape[1], 8) for c in range(0, src.shape[2], 512)]

        def gate_up(j0, j1, n):
            out = []
            for j in range(j0, j1):
                out += [rows32(wg_hbm, wg_buf, j, s_wg + n), rows32(wu_hbm, wu_buf, j, s_wu + n)]
            return out

        def tail_lists():
            gu = gate_up(_GU_HEAD, n_ffn, 1)
            dn = [rows32(wd_hbm, wd_buf, j, s_wd + sum(j * 32 >= r for r in d_bounds[1:]))
                  for j in range(n_ffn)]
            n_lo_gu = (len(gu) + len(dn) + _LAG) // 2 - len(dn)
            return gu[n_lo_gu:], gu[:n_lo_gu] + dn

        def issue_unit(i, w, next_lo):
            start_pairs(kv_list(i, w, 0, 0, n_kv), kv_list(i, w, 1, _LAG, n_kv) + next_lo)

        head = [(c_hbm, c_buf, s_c), (x_hbm, x_buf, s_x)]
        head += _merge(quads(wm_hbm, wm_buf, s_wm), gate_up(0, _GU_HEAD, 0))
        head += _merge(quads(wq_hbm, wq_buf, s_wq), quads(wo_hbm, wo_buf, s_wo))
        head_hi, head_lo = head[0::2], head[1::2]
        start_pairs([], head_lo[:_LAG])
        start_pairs(head_hi, head_lo[_LAG:] + kv_list(0, 0, 1, 0, _LAG))
        issue_unit(0, 0, kv_list(0, 1, 1, 0, _LAG))

        wait_filled(c_buf, s_c)
        wait_filled(x_buf, s_x)
        wait_filled(wm_buf, s_wm)

        def mod_cols(c0, c1):
            cf = c_buf[...].astype(f32)
            silu_c = (cf * jax.nn.sigmoid(cf)).astype(bf16)
            w = wm_buf[:, :, c0:c1].reshape(_D, c1 - c0)
            return jnp.dot(silu_c, w, preferred_element_type=f32)

        mod_a = mod_cols(0, 2 * _D)
        shift_a = mod_a[:, 0:_D]
        scale_a = mod_a[:, _D:2 * _D]
        h_scr[...] = (_layernorm(x_buf[...].astype(f32)) * (1.0 + scale_a) + shift_a).astype(bf16)

        def heads_of(half):
            return [(_OFF + 8 * block_of(half * _B, j // 8) + j % 8) % _H for j in range(_HU)]

        def head_rows(h):
            return pl.ds(pad + h, _B, stride=_H)

        def q_proj(half):
            hs = heads_of(half)
            w = jnp.concatenate(
                [wq_buf[:, :, h * _DH:(h + 1) * _DH].reshape(_D, _DH) for h in hs], axis=-1)
            q = jnp.dot(h_scr[...], w, preferred_element_type=f32).astype(bf16).astype(f32)
            for j, h in enumerate(hs):
                q_scr[head_rows(h), :] = q[:, j * _DH:(j + 1) * _DH]
                if h < _OFF:
                    q_scr[pad + _NW + h:pad + _NW + h + 1, :] = q[0:1, j * _DH:(j + 1) * _DH]

        def o_proj(half):
            hs = heads_of(half)
            oc = jnp.concatenate([o_scr[head_rows(h), :] for h in hs], axis=-1)
            w = jnp.concatenate(
                [wo_buf[h // 8, (h % 8) * _DH:(h % 8 + 1) * _DH, :] for h in hs], axis=0)
            return jnp.dot(oc.astype(bf16), w, preferred_element_type=f32)

        wait_filled(wq_buf, s_wq)
        wait_filled(wo_buf, s_wo)
        q_proj(0)

        row_s = lax.broadcasted_iota(jnp.int32, (8, win), 0)
        row_o = lax.broadcasted_iota(jnp.int32, (8, _DH), 0)

        def body(i, carry):
            slot = i % 2
            rows8 = [pl.ds(pl.multiple_of(8 + 8 * block_of(i, t), 8), 8) for t in range(2)]

            @pl.when(i + 1 < _NI)
            def _():
                issue_unit(i, 1, kv_list(i + 1, 0, 1, 0, _LAG))

            @pl.when(i + 1 == _NI)
            def _():
                issue_unit(_NI - 1, 1, tail_lists()[1][:_LAG])

            wait_filled(kbuf.at[slot], s_k + slot)
            for t in range(2):
                q8 = q_scr[rows8[t], :].astype(bf16)
                s_all = jnp.zeros((8, win), f32)
                for j in range(8):
                    s = lax.dot_general(q8, kbuf[slot, t * 8 + j], _NT, preferred_element_type=f32)
                    s_all = jnp.where(row_s == j, s, s_all)
                s_all = s_all * scale
                m = jnp.max(s_all, axis=-1, keepdims=True)
                p = jnp.exp(s_all - m)
                l_scr[t] = jnp.broadcast_to(jnp.sum(p, axis=-1, keepdims=True), (8, _DH))
                p_scr[t] = p

            @pl.when(i + 2 < _NI)
            def _():
                issue_unit(i + 1, 0, kv_list(i + 1, 1, 1, 0, _LAG))

            @pl.when(i + 2 == _NI)
            def _():
                issue_unit(_NI - 1, 0, kv_list(_NI - 1, 1, 1, 0, _LAG))

            @pl.when(i + 1 == _NI)
            def _():
                tail_hi, tail_lo = tail_lists()
                start_pairs(tail_hi, tail_lo[_LAG:])

            wait_filled(vbuf.at[slot], s_v + slot)
            for t in range(2):
                pb = p_scr[t].astype(bf16)
                o_all = jnp.zeros((8, _DH), f32)
                for j in range(8):
                    o = jnp.dot(pb, vbuf[slot, t * 8 + j], preferred_element_type=f32)
                    o_all = jnp.where(row_o == j, o, o_all)
                o_scr[rows8[t], :] = o_all / l_scr[t]

            @pl.when(i == 1)
            def _():
                mod_scr[...] = mod_cols(2 * _D, 6 * _D)

            @pl.when(i == 2)
            def _():
                q_proj(1)

            @pl.when(i == _B)
            def _():
                acc_scr[...] = o_proj(0)

            return carry

        lax.fori_loop(0, _NI, body, 0)

        o_scr[pad:8, :] = o_scr[pad + _NW:8 + _NW, :]
        gate_a = mod_scr[:, 0:_D]
        shift_b = mod_scr[:, _D:2 * _D]
        scale_b = mod_scr[:, 2 * _D:3 * _D]
        gate_b = mod_scr[:, 3 * _D:4 * _D]
        x1 = x_buf[...].astype(f32) + gate_a * (acc_scr[...] + o_proj(1))
        h2 = (_layernorm(x1) * (1.0 + scale_b) + shift_b).astype(bf16)
        for n in range(len(gu_bounds) - 1):
            r0, r1 = gu_bounds[n], gu_bounds[n + 1]
            wait_filled(wg_buf.at[r0:r1, :], s_wg + n)
            wait_filled(wu_buf.at[r0:r1, :], s_wu + n)
            gt = lax.dot_general(h2, wg_buf[r0:r1, :], _NT, preferred_element_type=f32)
            up = lax.dot_general(h2, wu_buf[r0:r1, :], _NT, preferred_element_type=f32)
            act_scr[:, r0:r1] = jax.nn.sigmoid(gt) * up
        for n in range(len(d_bounds) - 1):
            r0, r1 = d_bounds[n], d_bounds[n + 1]
            wait_filled(wd_buf.at[r0:r1, :], s_wd + n)
            y = jnp.dot(act_scr[:, r0:r1].astype(bf16), wd_buf[r0:r1, :], preferred_element_type=f32)
            if n == 0:
                acc_scr[...] = x1 + gate_b * y
            elif n < len(d_bounds) - 2:
                acc_scr[...] += gate_b * y
            else:
                o_ref[...] = (acc_scr[...] + gate_b * y).astype(o_ref.dtype)

    return kernel, n_sem


@jax.jit
def pallas_adaLN_cond__sliding_block_cached__glu_gated_glu__decode_kernel(
    A_x: jax.Array,
    A_k_cache: jax.Array,
    A_v_cache: jax.Array,
    A_wq: jax.Array,
    A_wo: jax.Array,
    B_x: jax.Array,
    B_w_gate: jax.Array,
    B_w_up: jax.Array,
    B_w_down: jax.Array,
    c: jax.Array,
    w_mod: jax.Array,
):
    del B_x
    sk = A_k_cache.shape[2]
    win = min(4096, max(256, sk // 4))
    ffn = B_w_down.shape[0]
    assert A_x.shape == (_B, 1, _D) and A_k_cache.shape == (_B, _H, sk, _DH)
    assert win == 1024 and ffn == 1376
    bf16 = jnp.bfloat16
    f32 = jnp.float32
    kernel, n_sem = _make_kernel(sk, win, ffn)

    hbm = pl.BlockSpec(memory_space=pltpu.MemorySpace.HBM)
    out = pl.pallas_call(
        kernel,
        in_specs=[hbm] * 10,
        out_specs=pl.BlockSpec(memory_space=pltpu.MemorySpace.VMEM),
        out_shape=jax.ShapeDtypeStruct((_B, _D), A_x.dtype),
        scratch_shapes=[
            pltpu.VMEM((2, _HU, win, _DH), bf16),
            pltpu.VMEM((2, _HU, win, _DH), bf16),
            pltpu.VMEM((4, _D // 4, _H * _DH), bf16),
            pltpu.VMEM((4, _H * _DH // 4, _D), bf16),
            pltpu.VMEM((ffn, _D), bf16),
            pltpu.VMEM((ffn, _D), bf16),
            pltpu.VMEM((ffn, _D), bf16),
            pltpu.VMEM((4, _D // 4, 6 * _D), bf16),
            pltpu.VMEM((_B, _D), bf16),
            pltpu.VMEM((_B, _D), bf16),
            pltpu.VMEM((_NW + 8 + _H, _DH), f32),
            pltpu.VMEM((_NW + 8 + _H, _DH), f32),
            pltpu.VMEM((_B, _D), bf16),
            pltpu.VMEM((_B, _D), f32),
            pltpu.VMEM((_B, 4 * _D), f32),
            pltpu.VMEM((_B, ffn), f32),
            pltpu.VMEM((2, 8, win), f32),
            pltpu.VMEM((2, 8, _DH), f32),
            pltpu.SemaphoreType.DMA((n_sem,)),
        ],
        compiler_params=pltpu.CompilerParams(
            vmem_limit_bytes=64 * 1024 * 1024,
            disable_bounds_checks=True,
            disable_semaphore_checks=True,
        ),
    )(
        A_x.reshape(_B, _D),
        A_k_cache.reshape(_NW, sk, _DH),
        A_v_cache.reshape(_NW, sk, _DH),
        A_wq.reshape(4, _D // 4, _H * _DH),
        A_wo.reshape(4, _H * _DH // 4, _D),
        B_w_gate.T,
        B_w_up.T,
        B_w_down,
        c,
        w_mod.reshape(4, _D // 4, 6 * _D),
    )
    return out.reshape(A_x.shape)
```
